```python
import os as _os
_os.environ.setdefault("JAX_PLATFORMS", "cpu")
import jax
import jax.numpy as jnp

def _softmax(x, axis=-1):
    return jax.nn.softmax(x, axis=axis)
def _gelu(x):
    return jax.nn.gelu(x, approximate=True)
def _silu(x):
    return jax.nn.silu(x)
def _sigmoid(x):
    return jax.nn.sigmoid(x)
def _layernorm(x, axis=-1, eps=1e-5):
    m = jnp.mean(x, axis=axis, keepdims=True)
    v = jnp.var(x, axis=axis, keepdims=True)
    return (x - m) / jnp.sqrt(v + eps)
def _scatter_add(tgt, idx, src, axis=0):
    return tgt.at[idx].add(src)
def _segment_sum(src, seg, n):
    return jax.ops.segment_sum(src, seg, n)
class _Rng:
    def __init__(self, key):
        self._k = key
    def _next(self):
        self._k, sub = jax.random.split(self._k)
        return sub
    def normal(self, shape):
        return jax.random.normal(self._next(), shape, dtype=jnp.bfloat16)
    def randint(self, lo, hi, shape):
        return jax.random.randint(self._next(), shape, lo, hi, dtype=jnp.int32)
    def uniform(self, shape, lo=0.0, hi=1.0):
        return jax.random.uniform(self._next(), shape, jnp.bfloat16, lo, hi)
    def permutation(self, n):
        return jax.random.permutation(self._next(), n)


kernel_name = 'gated_mix__linear_kernel_hedgehog__glu_gated_bilinear__prompt'

def setup_inputs():
    _rng = _Rng(jax.random.key(int.from_bytes(__import__("os").urandom(4), "little")))
    _w = (lambda a: (lambda t: t.astype(jnp.bfloat16) if jnp.issubdtype(t.dtype, jnp.floating) else t)(jnp.asarray(a)))
    def _A_setup():
        B, S, D, H = 1, 2048, 512, 32
        Dh = D // H
        return {
            "x": _w((lambda *s: _rng.normal(s) * 0.05)(B, S, D)),
            "wqkv": _w((lambda *s: _rng.normal(s) * 0.8)(D, 3 * D)),
            "w_phi": _w((lambda *s: _rng.normal(s) * 0.8)(H, Dh, Dh) * (Dh ** -0.5)),
            "wo": _w((lambda *s: _rng.normal(s) * 0.05)(D, D)),
        }
    _A_in = _A_setup()

    def _B_setup():
        B, S, D, F = 1, 2048, 512, 1792
        return {
            "x": _w((lambda *s: _rng.normal(s) * 0.05)(B, S, D)),
            "w_gate": _w((lambda *s: _rng.normal(s) * 1.6)(D, F) * (D ** -0.5)),
            "w_up": _w((lambda *s: _rng.normal(s) * 1.6)(D, F) * (D ** -0.5)),
            "w_down": _w((lambda *s: _rng.normal(s) * 1.6)(F, D) * (F ** -0.5)),
        }
    _B_in = _B_setup()

    return {
        "A_x": _A_in["x"],
        "A_wqkv": _A_in["wqkv"],
        "A_w_phi": _A_in["w_phi"],
        "A_wo": _A_in["wo"],
        "B_x": _B_in["x"],
        "B_w_gate": _B_in["w_gate"],
        "B_w_up": _B_in["w_up"],
        "B_w_down": _B_in["w_down"],
        "gate_w": _w((lambda *s: _rng.normal(s) * 0.05)(512) * 16.0),
    }

def reference(A_x, A_wqkv, A_w_phi, A_wo, B_x, B_w_gate, B_w_up, B_w_down, gate_w):
    def _A_ref(x, wqkv, w_phi, wo):
        B, S, D = x.shape
        H = 32; Dh = D // H
        qkv = (lambda x, *d: x.transpose(*d))((x @ wqkv).reshape(B, S, 3, H, Dh), 2, 0, 3, 1, 4)
        q, k, v = qkv[0], qkv[1], qkv[2]
        pq = jnp.einsum("bhsd,hdf->bhsf", q, w_phi)
        pk = jnp.einsum("bhsd,hdf->bhsf", k, w_phi)
        phi_q = jnp.concatenate([_softmax(pq, axis=-1), _softmax(-pq, axis=-1)], axis=-1)
        phi_k = jnp.concatenate([_softmax(pk, axis=-1), _softmax(-pk, axis=-1)], axis=-1)
        kv = jnp.einsum("bhsf,bhsd->bhfd", phi_k, v)
        z  = jnp.einsum("bhsf->bhf", phi_k)
        num = jnp.einsum("bhqf,bhfd->bhqd", phi_q, kv)
        den = jnp.einsum("bhqf,bhf->bhq", phi_q, z)[..., None] + 1e-6
        o = num / den
        return (lambda x, *d: x.transpose(*d))(o, 0, 2, 1, 3).reshape(B, S, D) @ wo

    def _B_ref(x, w_gate, w_up, w_down):
        g = jnp.einsum("bsd,df->bsf", x, w_gate)
        u = jnp.einsum("bsd,df->bsf", x, w_up)
        h = g * u
        return jnp.einsum("bsf,fd->bsd", h, w_down)

    x = A_x
    g = _sigmoid((x * gate_w).sum(-1, keepdims=True))
    a = _A_ref(x, A_wqkv, A_w_phi, A_wo)
    b = _B_ref(x, B_w_gate, B_w_up, B_w_down)
    return g * a + (1 - g) * b
```

```python
import contextlib
import functools

import jax
import jax.numpy as jnp
from jax import lax
import jax.experimental.pallas as pl
import jax.experimental.pallas.tpu as pltpu

S, D, H, DH, F = 2048, 512, 32, 16, 1792
NG = 8
NT_DIMS = (((1,), (1,)), ((), ()))
f32, bf16, u32 = jnp.float32, jnp.bfloat16, jnp.uint32
LOG2E = 1.4426950408889634
TS = 512
HT = TS // 2
HD = D // 2
HF = F // 2
NTILE = S // TS


def _nt(a, b):
    return lax.dot_general(a, b, NT_DIMS, preferred_element_type=f32)


def _nn(a, b):
    return jnp.dot(a, b, preferred_element_type=f32)


def _iota(shape, dim):
    return lax.broadcasted_iota(jnp.int32, shape, dim)


def _r4(x):
    return pltpu.roll(x, 4, 0)


def _rcp(x):
    r = pl.reciprocal(x, approx=True)
    return r * (2.0 - x * r)


def _exps(p):
    mx = jnp.max(p, axis=0)
    mx = jnp.maximum(mx, _r4(mx))
    mn = jnp.min(p, axis=0)
    mn = jnp.minimum(mn, _r4(mn))
    ep = jnp.exp2(p - mx[None])
    en = jnp.exp2(mn[None] - p)
    sp = jnp.sum(ep, axis=0)
    sp = sp + _r4(sp)
    sn = jnp.sum(en, axis=0)
    sn = sn + _r4(sn)
    return ep, en, _rcp(sp), _rcp(sn)


def _pk(t):
    return pltpu.bitcast(t, u32)


def _upk(t):
    return pltpu.bitcast(t, bf16)


def _zero_dep(tok):
    t = pltpu.bitcast(tok, u32)
    return pltpu.bitcast(lax.shift_right_logical(lax.shift_right_logical(t, u32(16)), u32(16)), f32)


def _gated(w, z):
    return (w.astype(f32).reshape(2, 8, 128) + z[None]).reshape(16, 128)


def _lhs7(a11, a12, a21, a22):
    return [a11 + a22, a21 + a22, a11, a22, a11 + a12, a21 - a11, a12 - a22]


def _rhs7(b11, b12, b21, b22):
    return [b11 + b22, b11, b12 - b22, b21 - b11, b22, b11 + b12, b21 + b22]


def _out4(m):
    m1, m2, m3, m4, m5, m6, m7 = m
    return m1 + m4 - m5 + m7, m3 + m5, m2 + m4, m1 - m2 + m3 + m6


_LHS_CHAIN = [((0, 0), [(2, "self")]), ((1, 0), [(5, ("-", (0, 0)))]), ((0, 1), [(4, ("+", (0, 0)))]),
              ((1, 1), [(0, ("+", (0, 0))), (3, "self")]), ((0, 1), [(6, ("-", (1, 1)))]),
              ((1, 0), [(1, ("+", (1, 1)))])]
_RHS_CHAIN = [((0, 0), [(1, "self")]), ((1, 0), [(3, ("-", (0, 0)))]), ((0, 1), [(5, ("+", (0, 0)))]),
              ((1, 1), [(0, ("+", (0, 0))), (4, "self")]), ((0, 1), [(2, ("-", (1, 1)))]),
              ((1, 0), [(6, ("+", (1, 1)))])]
_STEP_AT = (0, 1, 2, 3, 5, 6)
_SIDX = {0: 0, 1: 1, 4: 2, 5: 3, 6: 4}
_TIDX = {0: 0, 2: 1, 3: 2, 5: 3, 6: 4}
_MORD = (2, 4, 1, 3, 0, 6, 5)
_PAIRS = ((0, 1), (2, 3), (4, 5), (6, 7), (8, 9), (10, 11), (12, 13), (14, 15))


def _piece2(get, chain, f7, store, zs):
    held = {}
    for (Q, outs), z in zip(chain, zs):
        A, B = Q
        cur = [get(2 * A + a, 2 * B + b, z) for a in range(2) for b in range(2)]
        if Q in ((0, 0), (1, 1)):
            held[Q] = cur
        for sub, kind in outs:
            if kind == "self":
                o = cur
            elif kind[0] == "+":
                o = [c + h for c, h in zip(cur, held[kind[1]])]
            else:
                o = [c - h for c, h in zip(cur, held[kind[1]])]
            for j, v in enumerate(f7(*o)):
                store(sub * 7 + j, v.astype(bf16))


class _Pool:
    def __init__(self):
        self.items, self.total = [], 0

    def add(self, arr, cycles):
        self.items.append((arr, self.total, cycles))
        self.total += cycles

    def tok(self, frac):
        pos = frac * self.total
        for arr, start, cyc in self.items:
            if pos < start + cyc:
                nrb, ncb = arr.shape[0] // 8, arr.shape[1] // 128
                cb, rb = divmod(int((pos - start) / cyc * nrb * ncb), nrb)
                return _zero_dep(arr[rb * 8:rb * 8 + 8, cb * 128:cb * 128 + 128])
        raise ValueError(frac)


def _run_jobs(jobs, pool, lo=0.0, hi=0.98):
    tot = sum(j[0] for j in jobs)
    acc = 0
    for c, fn, nst in jobs:
        if nst:
            fn([pool.tok(lo + (hi - lo) * (acc + c * s / 7.0) / tot) for s in _STEP_AT])
        else:
            fn(pool.tok(lo + (hi - lo) * acc / tot))
        acc += c


def _mix(a, b):
    out, ia, ib = [], 0, 0
    while ia < len(a) or ib < len(b):
        if ib >= len(b) or (ia < len(a) and ia * len(b) <= ib * len(a)):
            out.append(a[ia])
            ia += 1
        else:
            out.append(b[ib])
            ib += 1
    return out


def make(X0=384, X1=256, T0F=0.7, BCUT=(32, 64, 72, 80, 84, 84), VW=(1, 1, 1, 0, 1), QFP=2, RSP=(48, 48, 32), RS2=2, NDPOS=20,
         OSPL=(128, 64, 32, 32), GLO=0.08, GHI=0.98, QHI=0.45, SXLO=0.5, SXHI=0.98, GG=0.98, NV3=5, PHI=0.4,
         views=True, scopes=False):
    X2 = X0 + X1
    P = functools.partial

    def scope(name):
        return jax.named_scope(name) if scopes else contextlib.nullcontext()

    def kernel(x_hbm, wqkv_hbm, wphi_hbm, wo_hbm, wg_hbm, wu_hbm, wd_hbm, gw_hbm, out_hbm,
               x_v, wqkv_v, wphi_v, wo_v, wg_v, wu_v, wd_v, gw_v, out_v,
               wqT_v, wkvT_v, kv_v, z_v, L_v, sx_v, tgu_v, td2_v, tdl_v, h2_v, pq_v, s1_v, two_v, tkv_v, sems):

        def rd(ref, lead, lo=None, hi=None):
            if lo is None:
                lo, hi = 0, ref.shape[-2]
            if views:
                return _upk(ref.bitcast(u32)[lead + (slice(lo // 2, hi // 2), slice(None))])
            return ref[lead + (slice(lo, hi), slice(None))]

        def rd2(ref, lead, n, lo=None, hi=None):
            return jnp.concatenate([rd(ref, lead + (j,), lo, hi) for j in range(n)], axis=1)

        def cp(src, dst, k):
            return pltpu.make_async_copy(src, dst, sems.at[k])

        def cx(r0, n, k):
            return cp(x_hbm.at[0, pl.ds(r0, n)], x_v.at[pl.ds(r0, n)], k)

        def cw(j, k):
            return cp(wqkv_hbm.at[:, pl.ds(j * D, D)], wqkv_v.at[:, pl.ds(j * D, D)], k)

        def co(r0, n):
            return cp(out_v.at[pl.ds(r0, n)], out_hbm.at[0, pl.ds(r0, n)], 6)

        c_wphi = cp(wphi_hbm, wphi_v, 0)
        c_wk = cw(1, 1)
        c_x0 = cx(0, X0, 2)
        c_x1 = cx(X0, X1, 3)
        c_wv = cw(2, 3)
        mid = [cx(X2, S - X2, 4), cw(0, 4), cp(gw_hbm, gw_v.at[pl.ds(0, D)], 4)]
        late = [cp(wg_hbm, wg_v, 5), cp(wu_hbm, wu_v, 5), cp(wd_hbm, wd_v, 5), cp(wo_hbm, wo_v, 5)]

        c_wphi.start()
        c_wk.start()
        c_x0.start()
        c_x1.start()
        c_wv.start()

        with scope("A"):
            Sm = (_iota((32, D), 1) // 16 == _iota((32, D), 0)).astype(bf16)
            m1 = _iota((256, D), 0) // 16 == _iota((256, D), 1) % 16
            Gm = ((_iota((128, 256), 0) % 64) // 4 == _iota((128, 256), 1) % 16).astype(bf16)
            r = _iota((128, D), 0)
            m2 = (r // 64) * 4 + r % 4 == (_iota((128, D), 1) // 16) % 8
            c_wphi.wait()
            R = wphi_v[...].reshape(256, 32)
            Xm = jnp.where(m1, _nn(R, Sm), 0.0).astype(bf16)
            A = jnp.where(m2, _nn(Gm, Xm), 0.0).astype(bf16)

        def fold(col0):
            return [LOG2E * _nt(A[:, g * 128:(g + 1) * 128], wqkv_v[:, col0 + g * 128:col0 + (g + 1) * 128])
                    for g in range(4)]

        def proj(r0, ts, w):
            return _nt(_upk(wkvT_v[w * HD:(w + 1) * HD, :]), x_v[r0:r0 + ts, :])

        def feat_k(p, z=None):
            p = p.reshape(8, 8, 128)
            if z is not None:
                p = p + z[None]
            ep, en, rp, rn = _exps(p)
            return jnp.concatenate([ep * rp[None], en * rn[None]], axis=0).reshape(128, 128)

        def soft_k(pT, tok=None):
            nc = pT.shape[1] // 128
            return [jnp.concatenate(
                [feat_k(pT[G * 64:(G + 1) * 64, c * 128:(c + 1) * 128], None if tok is None else tok(G * nc + c))
                 for c in range(nc)], axis=1).astype(bf16) for G in range(NG)]

        def kv_acc(vT, phis, first=False):
            ones = jnp.ones((16, vT.shape[1]), f32)
            for G in range(NG):
                lhs = jnp.concatenate([vT[G * 64:(G + 1) * 64, :], ones], axis=0).astype(bf16)
                kv = _nt(lhs, phis[G])[0:72]
                if first:
                    kv_v[G] = kv
                else:
                    kv_v[G] += kv

        def sx_piece(r0, rho, zs):
            def get(a, b, z):
                return _gated(x_v[pl.ds(r0 + a * 128 + rho * 16, 16), b * 128:(b + 1) * 128], z)

            def store(k, v):
                sx_v[k, rho * 16:(rho + 1) * 16, :] = v
            _piece2(get, _LHS_CHAIN, _lhs7, store, zs)

        def tgu_piece(rho, c, zs):
            def get(a, b, z):
                w_v = wg_v if b < 2 else wu_v
                c0 = (b % 2) * HF + c * 128
                return _gated(w_v[a * 128 + rho * 16:a * 128 + rho * 16 + 16, c0:c0 + 128], z)

            def store(k, v):
                tgu_v[k, c, rho * 16:(rho + 1) * 16, :] = v
            _piece2(get, _RHS_CHAIN, _rhs7, store, zs)

        def td2_piece(t, rho, zs):
            def get(a, b, z):
                r = (a // 2) * HF + (2 * t + a % 2) * 128 + rho * 16
                return _gated(wd_v[r:r + 16, b * 128:(b + 1) * 128], z)

            def store(k, v):
                td2_v[k, t * 128 + rho * 16:t * 128 + rho * 16 + 16, :] = v
            _piece2(get, _RHS_CHAIN, _rhs7, store, zs)

        def rhs1_piece(src, r_lo, r_hi, dst, rho, nq, z):
            q = [_gated(src[rr + rho * 16:rr + rho * 16 + 16, cc:cc + 128], z)
                 for rr in (r_lo, r_hi) for cc in (nq * 128, HD + nq * 128)]
            for k, v in enumerate(_rhs7(*q)):
                dst[k, nq, rho * 16:rho * 16 + 16, :] = v.astype(bf16)

        def s1_piece(pr, rho, kt, z):
            s = _lhs7(*[_gated(x_v[tb * 128 + rho * 16:tb * 128 + rho * 16 + 16, cc:cc + 128], z)
                        for tb in _PAIRS[pr] for cc in (kt * 128, HD + kt * 128)])
            for k, j in _SIDX.items():
                s1_v[pr, j, kt, rho * 16:rho * 16 + 16, :] = s[k].astype(bf16)

        def tkv_piece(w, rho, kt, z):
            r = w * HD + rho * 8
            t = _rhs7(*[_gated(_upk(wkvT_v[rr:rr + 8, cc:cc + 128]), z)
                        for cc in (kt * 128, HD + kt * 128) for rr in (r, r + 128)])
            for k, j in _TIDX.items():
                tkv_v[w, j, kt, rho * 16:rho * 16 + 16, :] = t[k].astype(bf16)

        def s1_jobs(prs):
            return [(1, P(s1_piece, pr, rho, kt), 0) for pr in prs for rho in range(8) for kt in range(2)]

        def qfold():
            fq = fold(0)
            for g, blk in enumerate(fq):
                wqT_v[g * 64:(g + 1) * 64, :] = _pk(blk.astype(bf16))
            gw = gw_v[pl.ds(0, D)].astype(f32).reshape(1, D)
            wqT_v[HD:HD + 8, :] = _pk(jnp.broadcast_to(gw, (16, D)).astype(bf16))
            return fq

        def s_rhs(pr, k):
            ta, tb = _PAIRS[pr]
            if k == 2:
                return x_v[ta * 128:(ta + 1) * 128, 0:HD]
            if k == 3:
                return x_v[tb * 128:(tb + 1) * 128, HD:D]
            return rd2(s1_v, (pr, _SIDX[k]), 2)

        cnt = [0]

        def sproj_unit(lhs_of, pr, pool):
            mm = [None] * 7
            for k in _MORD:
                mm[k] = _nt(lhs_of(k), s_rhs(pr, k))
                if cnt[0] % 2 == 0:
                    pool.add(mm[k][0:128], 128)
                cnt[0] += 1
            return mm

        def kv_unit(w, pr, rb, pool):
            def lhs_of(k):
                if k == 1:
                    return _upk(wkvT_v[w * HD + rb * 64:w * HD + (rb + 1) * 64, 0:HD])
                if k == 4:
                    return _upk(wkvT_v[w * HD + 128 + rb * 64:w * HD + 128 + (rb + 1) * 64, HD:D])
                return rd2(tkv_v, (w, _TIDX[k]), 2, rb * 128, (rb + 1) * 128)
            return _out4(sproj_unit(lhs_of, pr, pool))

        with scope("B"):
            c_wk.wait()
            for c in mid:
                c.start()
            for g, blk in enumerate(fold(D)):
                wkvT_v[g * 64:(g + 1) * 64, :] = _pk(blk.astype(bf16))
        with scope("C"):
            c_x0.wait()
            for c in late:
                c.start()
            p0 = proj(0, X0, 0)
        with scope("D"):
            c_x1.wait()
            c_wv.wait()
            p1 = proj(X0, X1, 0)
            wkvT_v[HD:D, :] = _pk(wqkv_v[:, 2 * D:3 * D].T)
            ph1 = soft_k(p1)
            v0 = proj(0, X0, 1)
            pool = _Pool()
            pool.add(v0, 1)
            ph0 = soft_k(p0, lambda j: pool.tok(T0F * j / (NG * (X0 // 128))))
            kv_acc(v0, ph0, True)
            v1 = proj(X0, X1, 1)
            pool = _Pool()
            pool.add(v1, 1)
            _run_jobs([(1, P(tkv_piece, w, rho, kt), 0) for w in range(2) for rho in range(16) for kt in range(2)], pool)
            prev = (v1, ph1)

        with scope("E"):
            for c in mid:
                c.wait()
            pool = _Pool()
            pk = proj(X2, 768 - X2, 0)
            pool.add(pk, (768 - X2) * 4)
            kv_acc(*prev)
            ph = soft_k(pk)
            vv = proj(X2, 768 - X2, 1)
            pool.add(vv, (768 - X2) * 4)
            prev = (vv, ph)
            allb = (s1_jobs(range(3, 8)) + [(8, P(sx_piece, 0, rho), 6) for rho in range(8)])
            cuts = [0] + list(BCUT) + [len(allb)]
            _run_jobs(allb[cuts[0]:cuts[1]], pool)
            phi = {}
            vblk = {}

            def soft_job(key, p, z):
                phi[key] = feat_k(p, z)

            def v_unit(u, pool):
                pr, rb = 3 + u // 2, u % 2
                for q, blk in enumerate(kv_unit(1, pr, rb, pool)):
                    vblk[(q % 2) * 2 + rb, _PAIRS[pr][q // 2]] = blk

            def kv_blocks(tbs):
                phis = [jnp.concatenate([phi[G, t] for t in tbs], axis=1).astype(bf16) for G in range(NG)]
                vT = jnp.concatenate([jnp.concatenate([vblk[nb, t] for t in tbs], axis=1) for nb in range(4)], axis=0)
                kv_acc(vT, phis)

            pend = []
            pool = _Pool()
            nv = 0
            for w in range(5):
                new_jobs = []
                pr = 3 + w
                for rb in range(2):
                    for q, blk in enumerate(kv_unit(0, pr, rb, pool)):
                        for hg in range(2):
                            key = ((q % 2) * 4 + rb * 2 + hg, _PAIRS[pr][q // 2])
                            new_jobs.append((4, P(soft_job, key, blk[hg * 64:(hg + 1) * 64]), 0))
                    if w == 0 and rb == 0:
                        kv_acc(*prev)
                _run_jobs(_mix(pend, allb[cuts[w + 1]:cuts[w + 2]]), pool)
                pend = new_jobs
                pool = _Pool()
                for _ in range(VW[w]):
                    v_unit(nv, pool)
                    nv += 1
            for j in range(NV3):
                v_unit(nv, pool)
                nv += 1
                if j == QFP:
                    for f in qfold():
                        pool.add(f, 128)
            _run_jobs(pend, pool, 0.0, PHI)
            _run_jobs(allb[cuts[6]:], pool, PHI, 0.98)
            kv_blocks((6, 7, 8, 9))

        with scope("G"):
            for c in late:
                c.wait()
            pool = _Pool()
            while nv < 10:
                v_unit(nv, pool)
                nv += 1
            for t in range(8):
                pq = _nt(_upk(wqT_v[0:HD + 8, :]), x_v[t * 256:(t + 1) * 256, :])
                pq_v[:, t * 256:(t + 1) * 256] = pq[0:D + 8]
                pool.add(pq[0:D], 1056)
                if t == 0:
                    kv_blocks((10, 11, 12))
                    kv_blocks((13, 14, 15))
            big = ([(7, P(tgu_piece, p % 8, p // 8), 6) for p in range(56)]
                   + [(7, P(td2_piece, p // 8, p % 8), 6) for p in range(24)])
            small = ([(1, P(rhs1_piece, wd_v, 6 * 128, HF + 6 * 128, tdl_v, q // 2, q % 2), 0) for q in range(16)]
                     + [(1, P(rhs1_piece, wo_v, 0, HD, two_v, q // 2, q % 2), 0) for q in range(32)])
            _run_jobs(_mix(big, small), pool, 0.0, GG)
            m_kv = _iota((64, 128), 0) // 16 == _iota((64, 128), 1) % 4
            for G in range(NG):
                z_v[G] = jnp.broadcast_to(kv_v[G, 64:72, :][None], (16, 8, 128)).reshape(128, 128).T
                L_v[G] = jnp.where(m_kv, kv_v[G, 0:64, :], 0.0).astype(bf16)

        def phase2(i, carry):
            r0 = pl.multiple_of(i * TS, TS)
            RO = [sum(RSP[:j]) for j in range(len(RSP))]
            RS = len(RSP)
            dz = lax.shift_right_logical(i, 8)

            def lane(c):
                return pl.ds(pl.multiple_of(r0 + c * 128, 128), 128)

            def q_soft(pool, hi):
                gs = [jax.nn.sigmoid(pq_v[D:D + 8, lane(c)]) for c in range(4)]
                phis = []
                for G in range(NG):
                    zp = z_v[G, 0:64, :].reshape(8, 8, 128)
                    zn = z_v[G, 64:128, :].reshape(8, 8, 128)
                    cols = []
                    for c in range(4):
                        p = pq_v[G * 64:(G + 1) * 64, lane(c)].reshape(8, 8, 128)
                        p = p + pool.tok(hi * (G * 4 + c) / 32)[None]
                        ep, en, rp, rn = _exps(p)
                        d8 = jnp.sum(ep * zp, axis=0) * rp + jnp.sum(en * zn, axis=0) * rn
                        rd_ = _rcp(d8 + _r4(d8) + 1e-6) * gs[c]
                        cols.append(jnp.concatenate([ep * (rp * rd_)[None], en * (rn * rd_)[None]],
                                                    axis=0).reshape(128, 128))
                    phis.append(jnp.concatenate(cols, axis=1).astype(bf16))
                omg = jnp.concatenate(
                    [jnp.broadcast_to((1.0 - g)[None], (16, 8, 128)).reshape(128, 128).T for g in gs], axis=0)
                return phis, omg

            def q_out(phis):
                oT = jnp.concatenate([_nn(L_v[G], phis[G]) for G in range(NG)], axis=0)
                cmb = _lhs7(oT[0:HD, 0:HT], oT[HD:D, 0:HT], oT[0:HD, HT:TS], oT[HD:D, HT:TS])
                return [c.T.astype(bf16) for c in cmb]

            def gu_unit(c, rsi, pool):
                mo = []
                for a in range(7):
                    mm = [_nn(rd(sx_v, (a * 7 + b,), RO[rsi], RO[rsi] + RSP[rsi]), rd(tgu_v, (a * 7 + b, c)))
                          for b in range(7)]
                    for m in mm:
                        pool.add(m[0:8], 1)
                    mo.append(_out4(mm))
                cblk = [_out4([mo[a][q] for a in range(7)]) for q in range(4)]
                return [[cblk[(r % 2) * 2 + n][(r // 2) * 2] * cblk[(r % 2) * 2 + n][(r // 2) * 2 + 1]
                         for n in range(2)] for r in range(4)]

            def h2_piece(blk, t, row, ps, zs):
                def get(a, b, z):
                    return _gated(blk[a][b][ps * 16:ps * 16 + 16, :], z)

                def store(k, v):
                    h2_v[k, t, row + ps * 16:row + ps * 16 + 16, :] = v
                _piece2(get, _LHS_CHAIN, _lhs7, store, zs)

            pend = []
            for t in range(3):
                for rsi in range(RS):
                    pool = _Pool()
                    ha, hb = gu_unit(2 * t, rsi, pool), gu_unit(2 * t + 1, rsi, pool)
                    _run_jobs(pend, pool, GLO, GHI)
                    blk = [[ha[r][0], hb[r][0], ha[r][1], hb[r][1]] for r in range(4)]
                    pend = [(7, P(h2_piece, blk, t, RO[rsi], ps), 6) for ps in range(RSP[rsi] // 16)]
            pool = _Pool()
            hl = []
            for rsi in range(RS):
                hc = gu_unit(6, rsi, pool)
                hl.append([_lhs7(hc[rp][0], hc[rp][1], hc[2 + rp][0], hc[2 + rp][1]) for rp in range(2)])
            _run_jobs(pend, pool, GLO * 2 / RS, GHI * 2 / RS)
            hlf = [[jnp.concatenate([hl[rsi][rp][a] for rsi in range(RS)], axis=0) for a in range(7)]
                   for rp in range(2)]

            DW = 128 // RS2
            NP = 49 * RS2
            nq = int(QHI * NP)
            units = []
            pool = _Pool()
            st = {}
            for u in range(RS2):
                mo = []
                for a in range(7):
                    mm = []
                    for b in range(7):
                        k = a * 7 + b
                        mm.append(_nn(rd2(h2_v, (k + dz,), 3, u * DW, (u + 1) * DW), rd(td2_v, (k,))))
                        pool.add(mm[-1][0:8], 1)
                        if pool.total == nq:
                            st["q"] = q_soft(pool, 1.0)
                        if pool.total == nq + (NDPOS * NP) // 98:
                            st["o"] = q_out(st["q"][0])
                    inner = _out4(mm)
                    lhs = jnp.concatenate([hlf[rp][a][u * DW:(u + 1) * DW] for rp in range(2)], axis=0)
                    ml = _nn(lhs.astype(bf16), rd2(tdl_v, (a,), 2))
                    mo.append([inner[rp * 2 + n] + ml[rp * DW:(rp + 1) * DW, n * 128:(n + 1) * 128]
                               for rp in range(2) for n in range(2)])
                cblk = [_out4([mo[a][q] for a in range(7)]) for q in range(4)]
                units.append([jnp.concatenate([cblk[(r % 2) * 2 + nb % 2][(r // 2) * 2 + nb // 2]
                                               for nb in range(4)], axis=1) for r in range(4)])
            rn0 = pl.multiple_of(jnp.minimum(i + 1, NTILE - 1) * TS, TS)
            _run_jobs([(7, P(sx_piece, rn0, rho), 6) for rho in range(8)], pool, SXLO, SXHI)
            o, omg = st["o"], st["q"][1]
            b = jnp.concatenate([units[u][r] for r in range(4) for u in range(RS2)], axis=0)
            s0 = 0
            for n in OSPL:
                m = [None] * 7
                for k in (2, 4, 0, 3, 6, 1, 5):
                    m[k] = _nn(o[k][s0:s0 + n], rd2(two_v, (k,), 2))
                for half in range(2):
                    rh = slice(half * HT + s0, half * HT + s0 + n)
                    om = jnp.concatenate([omg[rh]] * 2, axis=1)
                    bl, br = om * b[rh, 0:HD], om * b[rh, HD:D]
                    if half == 0:
                        ol, orr = bl + m[0] + m[3] - m[4] + m[6], br + m[2] + m[4]
                    else:
                        ol, orr = bl + m[3] + m[1], br + m[2] + m[0] - m[1] + m[5]
                    out_v[pl.ds(r0 + half * HT + s0, n), :] = jnp.concatenate([ol, orr], axis=1).astype(bf16)
                    co(r0 + half * HT + s0, n).start()
                s0 += n
            return carry

        with scope("phase2"):
            lax.fori_loop(0, NTILE, phase2, 0)
        co(0, S).wait()

    @jax.jit
    def fn(A_x, A_wqkv, A_w_phi, A_wo, B_x, B_w_gate, B_w_up, B_w_down, gate_w):
        any_spec = pl.BlockSpec(memory_space=pl.ANY)
        return pl.pallas_call(
            kernel,
            in_specs=[any_spec] * 8,
            out_specs=any_spec,
            out_shape=jax.ShapeDtypeStruct((1, S, D), bf16),
            scratch_shapes=[
                pltpu.VMEM((S, D), bf16),
                pltpu.VMEM((D, 3 * D), bf16),
                pltpu.VMEM((DH, DH, H), bf16),
                pltpu.VMEM((D, D), bf16),
                pltpu.VMEM((D, F), bf16),
                pltpu.VMEM((D, F), bf16),
                pltpu.VMEM((F, D), bf16),
                pltpu.VMEM((8192,), bf16),
                pltpu.VMEM((S, D), bf16),
                pltpu.VMEM((HD + 8, D), u32),
                pltpu.VMEM((D, D), u32),
                pltpu.VMEM((NG, 72, 128), f32),
                pltpu.VMEM((NG, 128, 128), f32),
                pltpu.VMEM((NG, 64, 128), bf16),
                pltpu.VMEM((49, 128, 128), bf16),
                pltpu.VMEM((49, 7, 128, 128), bf16),
                pltpu.VMEM((49, 384, 128), bf16),
                pltpu.VMEM((7, 2, 128, 128), bf16),
                pltpu.VMEM((49, 4, 128, 128), bf16),
                pltpu.VMEM((D + 8, S), f32),
                pltpu.VMEM((8, 5, 2, 128, 128), bf16),
                pltpu.VMEM((7, 2, HD, 128), bf16),
                pltpu.VMEM((2, 5, 2, HD, 128), bf16),
                pltpu.SemaphoreType.DMA((7,)),
            ],
            compiler_params=pltpu.CompilerParams(
                vmem_limit_bytes=100 * 1024 * 1024,
                disable_bounds_checks=True, disable_semaphore_checks=True),
        )(A_x, A_wqkv, A_w_phi.transpose(1, 2, 0), A_wo, B_w_gate, B_w_up, B_w_down, gate_w)

    return fn


_impl = make()


@jax.jit
def pallas_gated_mix__linear_kernel_hedgehog__glu_gated_bilinear__prompt_kernel(
    A_x: jax.Array,
    A_wqkv: jax.Array,
    A_w_phi: jax.Array,
    A_wo: jax.Array,
    B_x: jax.Array,
    B_w_gate: jax.Array,
    B_w_up: jax.Array,
    B_w_down: jax.Array,
    gate_w: jax.Array,
):
    return _impl(A_x, A_wqkv, A_w_phi, A_wo, B_x, B_w_gate, B_w_up, B_w_down, gate_w)
```
